```python
import jax
import jax.numpy as jnp

def _softmax(x, axis=-1):
    return jax.nn.softmax(x, axis=axis)
def _gelu(x):
    return jax.nn.gelu(x, approximate=True)
def _silu(x):
    return jax.nn.silu(x)
def _sigmoid(x):
    return jax.nn.sigmoid(x)
def _layernorm(x, axis=-1, eps=1e-5):
    m = jnp.mean(x, axis=axis, keepdims=True)
    v = jnp.var(x, axis=axis, keepdims=True)
    return (x - m) / jnp.sqrt(v + eps)
def _scatter_add(tgt, idx, src, axis=0):
    return tgt.at[idx].add(src)
def _segment_sum(src, seg, n):
    return jax.ops.segment_sum(src, seg, n)
class _Rng:
    def __init__(self, key):
        self._k = key
    def _next(self):
        self._k, sub = jax.random.split(self._k)
        return sub
    def normal(self, shape):
        return jax.random.normal(self._next(), shape, dtype=jnp.bfloat16)
    def randint(self, lo, hi, shape):
        return jax.random.randint(self._next(), shape, lo, hi, dtype=jnp.int32)
    def uniform(self, shape, lo=0.0, hi=1.0):
        return jax.random.uniform(self._next(), shape, jnp.bfloat16, lo, hi)
    def permutation(self, n):
        return jax.random.permutation(self._next(), n)


kernel_name = 'standalone__detection_seg_fpn_lateral__vision'

def setup_inputs():
    _rng = _Rng(jax.random.key(int.from_bytes(__import__("os").urandom(4), "little")))
    _w = (lambda a: (lambda t: t.astype(jnp.bfloat16) if jnp.issubdtype(t.dtype, jnp.floating) else t)(jnp.asarray(a)))
    H = W = (384 // 2) * 2
    C = 384
    k = 1
    return {
        "c_fine": _w((lambda *s: _rng.normal(s) * 0.05)(1, H, W, C)),
        "p_coarse": _w((lambda *s: _rng.normal(s) * 0.05)(1, H // 2, W // 2, C)),
        "w_lat": _w((lambda *s: _rng.normal(s) * 0.05)(C, C)),
        "w_out": _w((lambda *s: _rng.normal(s) * 0.05)(k, k, C, C)),
    }

def reference(c_fine, p_coarse, w_lat, w_out):
    B, H, W, C = c_fine.shape
    k = 1
    lat = jnp.einsum("bhwc,cd->bhwd", c_fine, w_lat)
    up = jnp.repeat(jnp.repeat(p_coarse, 2, axis=1), 2, axis=2)
    m = lat + up
    pad = k // 2
    mp = jnp.pad(m, ((0, 0), (pad, pad), (pad, pad), (0, 0)))
    o = None
    for di in range(k):
        for dj in range(k):
            t = jnp.einsum("bhwc,cd->bhwd", mp[:, di:di + H, dj:dj + W, :], w_out[di, dj])
            o = t if o is None else o + t
    return o
```

```python
import jax
import jax.numpy as jnp
from jax import lax
import jax.experimental.pallas as pl
import jax.experimental.pallas.tpu as pltpu

_LANES = 128
_STREAMS = 6
_WRITE_ROWS = 48
_P_SLOTS = 14
_SWITCH_UNIT = 17
_PAIRS_PER_STEP = 2


@jax.jit
def pallas_standalone__detection_seg_fpn_lateral__vision_kernel(
    c_fine: jax.Array,
    p_coarse: jax.Array,
    w_lat: jax.Array,
    w_out: jax.Array,
):
    B, H, W, C = c_fine.shape
    S, K, U0 = _STREAMS, _P_SLOTS, _SWITCH_UNIT
    W2 = W // 2
    n = B * H // 2 // S
    pieces = 2 * W // _WRITE_ROWS
    assert n * S * 2 == B * H and pieces * _WRITE_ROWS == 2 * W
    assert K <= n and n - 1 - K <= U0 < n and S % _PAIRS_PER_STEP == 0
    dt = c_fine.dtype
    f32 = jnp.float32

    def kernel(c_hbm, p_hbm, wl_hbm, wo_hbm, o_hbm,
               cbuf, pbuf, wl, wo, wc, up, gsem, csem, psem, osem):
        def read_c(u):
            return pltpu.make_async_copy(c_hbm.at[:, u], cbuf.at[u], csem.at[u])

        def read_p(u):
            return pltpu.make_async_copy(
                p_hbm.at[:, u], pbuf.at[u % K], psem.at[u % K])

        def start_read(u, carry):
            read_p(u).start()
            read_c(u).start()
            return carry

        def wait_read(u, carry):
            read_p(u).wait()
            read_c(u).wait()
            return carry

        def start_write(u, carry):
            for j in range(pieces):
                rows = pl.ds(j * _WRITE_ROWS, _WRITE_ROWS)
                pltpu.make_async_copy(
                    cbuf.at[u, :, rows], o_hbm.at[:, u, rows], osem.at[u]).start()
            return carry

        def wait_write(u, carry):
            pltpu.make_async_copy(cbuf.at[u], cbuf.at[u], osem.at[u]).wait()
            return carry

        def compute_pair(u, s):
            q = jnp.dot(pbuf[u % K, s], wo[...], preferred_element_type=f32)
            for j in range(C // _LANES):
                qj = q[:, j * _LANES:(j + 1) * _LANES]
                up[j, pl.ds(0, W2, stride=2), :] = qj
                up[j, pl.ds(1, W2, stride=2), :] = qj
            q_up = jnp.concatenate([up[j] for j in range(C // _LANES)], axis=1)
            for t in range(2):
                rows = pl.ds(t * W, W)
                acc = jnp.dot(cbuf[u, s, rows], wc[...], preferred_element_type=f32)
                cbuf[u, s, rows] = (acc + q_up).astype(dt)

        copy_wl = pltpu.make_async_copy(wl_hbm, wl, gsem.at[0])
        copy_wo = pltpu.make_async_copy(wo_hbm, wo, gsem.at[1])
        copy_wl.start()
        copy_wo.start()
        lax.fori_loop(0, K, start_read, 0)
        copy_wl.wait()
        copy_wo.wait()
        wc[...] = jnp.dot(wl[...], wo[...], preferred_element_type=f32).astype(dt)

        def unit(u, carry):
            @pl.when(u <= U0)
            def _():
                wait_read(u, 0)

            def step(g, carry):
                for i in range(_PAIRS_PER_STEP):
                    compute_pair(u, g * _PAIRS_PER_STEP + i)
                return carry

            lax.fori_loop(0, S // _PAIRS_PER_STEP, step, 0)

            @pl.when(u + K < n)
            def _():
                start_read(u + K, 0)

            @pl.when(u == U0)
            def _():
                lax.fori_loop(U0 + 1, n, wait_read, 0)

            @pl.when(u >= U0)
            def _():
                def issued(x):
                    return jnp.minimum(x + 1, 3 + 2 * (x - U0))

                lo = jnp.where(u == U0, 0, issued(u - 1))
                hi = jnp.where(u == n - 1, n, issued(u))
                lax.fori_loop(lo, hi, start_write, 0)

            return carry

        lax.fori_loop(0, n, unit, 0)
        lax.fori_loop(0, n, wait_write, 0)

    out = pl.pallas_call(
        kernel,
        in_specs=[pl.BlockSpec(memory_space=pl.ANY)] * 4,
        out_specs=pl.BlockSpec(memory_space=pl.ANY),
        out_shape=jax.ShapeDtypeStruct((S, n, 2 * W, C), dt),
        scratch_shapes=[
            pltpu.VMEM((n, S, 2 * W, C), dt),
            pltpu.VMEM((K, S, W2, C), dt),
            pltpu.VMEM((C, C), dt),
            pltpu.VMEM((C, C), dt),
            pltpu.VMEM((C, C), dt),
            pltpu.VMEM((C // _LANES, W, _LANES), f32),
            pltpu.SemaphoreType.DMA((2,)),
            pltpu.SemaphoreType.DMA((n,)),
            pltpu.SemaphoreType.DMA((K,)),
            pltpu.SemaphoreType.DMA((n,)),
        ],
        compiler_params=pltpu.CompilerParams(vmem_limit_bytes=127 * 2**20),
    )(
        c_fine.reshape(S, n, 2 * W, C),
        p_coarse.reshape(S, n, W2, C),
        w_lat,
        w_out.reshape(C, C),
    )
    return out.reshape(B, H, W, C)
```

```python
import jax
import jax.numpy as jnp
from jax import lax
import jax.experimental.pallas as pl
import jax.experimental.pallas.tpu as pltpu

_LANES = 128
_MARK_ROWS = 16
_STREAMS = 6
_READ_PHASE_UNITS = 18
_LOOKAHEAD = 14
_CHUNK_ROWS = 96
_SMALL_READ_ROWS = 56
_WRITE_ROWS = 48
_HIGH, _LOW = 0, 1


@jax.jit
def pallas_standalone__detection_seg_fpn_lateral__vision_kernel(
    c_fine: jax.Array,
    p_coarse: jax.Array,
    w_lat: jax.Array,
    w_out: jax.Array,
):
    B, H, W, C = c_fine.shape
    S, NA, K, MC = _STREAMS, _READ_PHASE_UNITS, _LOOKAHEAD, _CHUNK_ROWS
    U, V = 2 * W, W // 2
    n = B * H // 2 // S
    rows_b = (n - NA) * U
    small_per_pair = (U + V) // MC
    bulk_b = rows_b - NA * small_per_pair * _SMALL_READ_ROWS
    assert 2 * n * S == B * H and S % 2 == 0 and V % MC == 0 and U % _WRITE_ROWS == 0
    assert K <= NA < n <= NA + K and bulk_b > 0 and bulk_b % 8 == 0
    dt = c_fine.dtype
    f32 = jnp.float32

    def kernel(c_hbm, p_hbm, wl_hbm, wo_hbm, o_hbm,
               buf_a, buf_b, buf_p, wl, wo, wc, up, w_sem, r_sem, b_sem, o_sem):

        def rows(u, size=U, offset=0):
            return pl.ds(pl.multiple_of(u * U + offset, 8), size)

        def loop(lo, hi, fn):
            def body(i, carry):
                fn(i)
                return carry

            lax.fori_loop(lo, hi, body, 0)

        def read_a(u):
            return pltpu.make_async_copy(
                c_hbm.at[:, rows(u)], buf_a.at[:, rows(u)], r_sem.at[u % K])

        def read_p(u):
            return pltpu.make_async_copy(
                p_hbm.at[:, u], buf_p.at[u % K], r_sem.at[u % K])

        def start_bulk_read(u):
            read_p(u).start(priority=_LOW)

            @pl.when(u < NA)
            def _():
                read_a(u).start(priority=_LOW)

            @pl.when(u == NA)
            def _():
                pltpu.make_async_copy(
                    c_hbm.at[:, pl.ds(NA * U, bulk_b)],
                    buf_b.at[:, pl.ds(0, bulk_b)],
                    b_sem.at[0],
                ).start(priority=_LOW)

        def start_small_read(s, i, result):
            buf_b[0, pl.ds(rows_b, _MARK_ROWS), pl.ds(0, _LANES)] = (
                result[MC - _MARK_ROWS:, C - _LANES:].astype(dt))
            at = pl.multiple_of(bulk_b + i * _SMALL_READ_ROWS, 8)
            pltpu.make_async_copy(
                c_hbm.at[s, pl.ds(NA * U + at, _SMALL_READ_ROWS)],
                buf_b.at[s, pl.ds(at, _SMALL_READ_ROWS)],
                b_sem.at[0],
            ).start(priority=_HIGH)

        def start_write(u):
            def pieces(buf, i, sem):
                for offset in range(0, U, _WRITE_ROWS):
                    pltpu.make_async_copy(
                        buf.at[:, rows(i, _WRITE_ROWS, offset)],
                        o_hbm.at[:, rows(u, _WRITE_ROWS, offset)],
                        sem,
                    ).start()

            pl.when(u < NA)(lambda: pieces(buf_a, u, o_sem.at[0]))
            pl.when(u >= NA)(lambda: pieces(buf_b, u - NA, o_sem.at[1]))

        def compute_pair(fine, coarse, chunk, after_chunk=None):
            step = 0
            coarse_chunk = min(chunk, V)
            for v in range(0, V, coarse_chunk):
                q = jnp.dot(coarse[pl.ds(v, coarse_chunk)], wo[...],
                            preferred_element_type=f32)
                for j in range(C // _LANES):
                    qj = q[:, j * _LANES:(j + 1) * _LANES]
                    up[j, pl.ds(2 * v, coarse_chunk, stride=2), :] = qj
                    up[j, pl.ds(2 * v + 1, coarse_chunk, stride=2), :] = qj
                if after_chunk is not None:
                    after_chunk(step, q)
                step += 1
            for r in range(0, U, chunk):
                q_up = jnp.concatenate(
                    [up[j, pl.ds(r % W, chunk), :] for j in range(C // _LANES)], axis=1)
                acc = jnp.dot(fine[pl.ds(r, chunk)], wc[...], preferred_element_type=f32)
                result = (acc + q_up).astype(dt)
                fine[pl.ds(r, chunk)] = result
                if after_chunk is not None:
                    after_chunk(step, result)
                step += 1

        copy_wl = pltpu.make_async_copy(wl_hbm, wl, w_sem.at[0])
        copy_wo = pltpu.make_async_copy(wo_hbm, wo, w_sem.at[0])
        copy_wl.start(priority=_LOW)
        copy_wo.start(priority=_LOW)
        loop(0, K, start_bulk_read)
        copy_wl.wait()
        copy_wo.wait()
        wc[...] = jnp.dot(wl[...], wo[...], preferred_element_type=f32).astype(dt)

        def read_phase_unit(u):
            read_p(u).wait()
            read_a(u).wait()
            loop(0, S, lambda s: compute_pair(
                buf_a.at[s, rows(u)],
                buf_p.at[u % K, s],
                MC,
                lambda k, res: start_small_read(s, u * small_per_pair + k, res)))
            pl.when(u + K < n)(lambda: start_bulk_read(u + K))

        loop(0, NA, read_phase_unit)

        data_b = buf_b.at[:, pl.ds(0, rows_b)]
        pltpu.make_async_copy(data_b, data_b, b_sem.at[0]).wait()
        loop(NA, n - 1, lambda u: read_p(u).wait())

        def writes_started(u):
            return jnp.minimum(u + 1, 3 + 13 * (u - NA + 1) // 6)

        loop(0, writes_started(NA - 1), start_write)
        read_p(n - 1).wait()

        def write_phase_unit(u):
            def two_pairs(g):
                for s in (2 * g, 2 * g + 1):
                    compute_pair(buf_b.at[s, rows(u - NA)], buf_p.at[u % K, s], W)

            loop(0, S // 2, two_pairs)
            loop(writes_started(u - 1),
                 jnp.where(u == n - 1, n, writes_started(u)),
                 start_write)

        loop(NA, n, write_phase_unit)
        pltpu.make_async_copy(buf_a, buf_a, o_sem.at[0]).wait()
        pltpu.make_async_copy(data_b, data_b, o_sem.at[1]).wait()

    out = pl.pallas_call(
        kernel,
        in_specs=[pl.BlockSpec(memory_space=pl.ANY)] * 4,
        out_specs=pl.BlockSpec(memory_space=pl.ANY),
        out_shape=jax.ShapeDtypeStruct((S, n * U, C), dt),
        scratch_shapes=[
            pltpu.VMEM((S, NA * U, C), dt),
            pltpu.VMEM((S, rows_b + _MARK_ROWS, C), dt),
            pltpu.VMEM((K, S, V, C), dt),
            pltpu.VMEM((C, C), dt),
            pltpu.VMEM((C, C), dt),
            pltpu.VMEM((C, C), dt),
            pltpu.VMEM((C // _LANES, W, _LANES), f32),
            pltpu.SemaphoreType.DMA((1,)),
            pltpu.SemaphoreType.DMA((K,)),
            pltpu.SemaphoreType.DMA((1,)),
            pltpu.SemaphoreType.DMA((2,)),
        ],
        compiler_params=pltpu.CompilerParams(vmem_limit_bytes=127 * 2**20),
    )(
        c_fine.reshape(S, n * U, C),
        p_coarse.reshape(S, n, V, C),
        w_lat,
        w_out.reshape(C, C),
    )
    return out.reshape(B, H, W, C)
```
